```python
import jax
import jax.numpy as jnp

def _softmax(x, axis=-1):
    return jax.nn.softmax(x, axis=axis)
def _gelu(x):
    return jax.nn.gelu(x, approximate=True)
def _silu(x):
    return jax.nn.silu(x)
def _sigmoid(x):
    return jax.nn.sigmoid(x)
def _layernorm(x, axis=-1, eps=1e-5):
    m = jnp.mean(x, axis=axis, keepdims=True)
    v = jnp.var(x, axis=axis, keepdims=True)
    return (x - m) / jnp.sqrt(v + eps)
def _scatter_add(tgt, idx, src, axis=0):
    return tgt.at[idx].add(src)
def _segment_sum(src, seg, n):
    return jax.ops.segment_sum(src, seg, n)
class _Rng:
    def __init__(self, key):
        self._k = key
    def _next(self):
        self._k, sub = jax.random.split(self._k)
        return sub
    def normal(self, shape):
        return jax.random.normal(self._next(), shape, dtype=jnp.bfloat16)
    def randint(self, lo, hi, shape):
        return jax.random.randint(self._next(), shape, lo, hi, dtype=jnp.int32)
    def uniform(self, shape, lo=0.0, hi=1.0):
        return jax.random.uniform(self._next(), shape, jnp.bfloat16, lo, hi)
    def permutation(self, n):
        return jax.random.permutation(self._next(), n)


kernel_name = 'sequential_preLN__sliding_block_cached__moe_arch_mod__decode'

def setup_inputs():
    _rng = _Rng(jax.random.key(int.from_bytes(__import__("os").urandom(4), "little")))
    _w = (lambda a: (lambda t: t.astype(jnp.bfloat16) if jnp.issubdtype(t.dtype, jnp.floating) else t)(jnp.asarray(a)))
    def _A_setup():
        B, Sq, D = 1, 1, 640
        Hq, Hkv, Sk, Dh = 32, 32, 32768, 192
        assert Hq % Hkv == 0, (Hq, Hkv)
        return {
            "x": _w((lambda *s: _rng.normal(s) * 0.05)(B, Sq, D)),
            "k_cache": _w((lambda *s: _rng.normal(s) * 0.05)(B, Hkv, Sk, Dh)),
            "v_cache": _w((lambda *s: _rng.normal(s) * 0.05)(B, Hkv, Sk, Dh)),
            "wq": _w((lambda *s: _rng.normal(s) * 0.05)(D, Hq * Dh) * (D ** -0.5)),
            "wo": _w((lambda *s: _rng.normal(s) * 0.05)(Hq * Dh, D) * ((Hq * Dh) ** -0.5)),
        }
    _A_in = _A_setup()

    def _B_setup():
        B, S, D, F, C = 1, 1, 640, 1536, 1
        return {
            "x": _w((lambda *s: _rng.normal(s) * 0.05)(B, S, D)),
            "w_r": _w((lambda *s: _rng.normal(s) * 0.05)(D)),
            "w_gate": _w((lambda *s: _rng.normal(s) * 0.05)(D, F)),
            "w_up": _w((lambda *s: _rng.normal(s) * 0.05)(D, F)),
            "w_down": _w((lambda *s: _rng.normal(s) * 0.05)(F, D)),
        }
    _B_in = _B_setup()

    return {
        "A_x": _A_in["x"],
        "A_k_cache": _A_in["k_cache"],
        "A_v_cache": _A_in["v_cache"],
        "A_wq": _A_in["wq"],
        "A_wo": _A_in["wo"],
        "B_x": _B_in["x"],
        "B_w_r": _B_in["w_r"],
        "B_w_gate": _B_in["w_gate"],
        "B_w_up": _B_in["w_up"],
        "B_w_down": _B_in["w_down"],
    }

def reference(A_x, A_k_cache, A_v_cache, A_wq, A_wo, B_x, B_w_r, B_w_gate, B_w_up, B_w_down):
    def _A_ref(x, k_cache, v_cache, wq, wo):
        B, Sq, D = x.shape
        Hq, Dh = 32, 192
        Hkv, Sk = k_cache.shape[1], k_cache.shape[2]
        W = min(4096, max(256, Sk // 4))
        rep = Hq // Hkv
        q = (lambda x, *d: x.transpose(*d))((x @ wq).reshape(B, Sq, Hq, Dh), 0, 2, 1, 3)
        k = jnp.repeat(k_cache[:, :, Sk - W:, :], rep, axis=1)
        v = jnp.repeat(v_cache[:, :, Sk - W:, :], rep, axis=1)
        scores = jnp.einsum("bhqd,bhkd->bhqk", q, k) * (Dh ** -0.5)
        p = _softmax(scores, axis=-1)
        o = jnp.einsum("bhqk,bhkd->bhqd", p, v)
        return (lambda x, *d: x.transpose(*d))(o, 0, 2, 1, 3).reshape(B, Sq, Hq * Dh) @ wo

    def _B_ref(x, w_r, w_gate, w_up, w_down):
        B, S, D = x.shape
        C = 1
        r = x @ w_r
        idx = jnp.argsort(-r, axis=-1)[:, :C]
        idx_e = jnp.repeat(idx.reshape(B, C, 1), D, axis=2)
        x_sel = jnp.take_along_axis(x, idx_e, axis=1)
        g = _silu(x_sel @ w_gate)
        u = x_sel @ w_up
        y = (g * u) @ w_down
        r_sel = _sigmoid(jnp.take_along_axis(r, idx, axis=1))
        y = y * r_sel.reshape(B, C, 1)
        b_off = (jnp.arange(B) * S).reshape(B, 1)
        flat_idx = (idx + b_off).reshape(B * C)
        zero = (x * 0.0).reshape(B * S, D)
        upd = _scatter_add(zero, flat_idx, y.reshape(B * C, D), axis=0)
        return x + upd.reshape(B, S, D)

    x = A_x
    h = x + _A_ref(_layernorm(x, axis=-1), A_k_cache, A_v_cache, A_wq, A_wo)
    h2 = h + _B_ref(_layernorm(h, axis=-1), B_w_r, B_w_gate, B_w_up, B_w_down)
    return h2
```

```python
import jax
import jax.numpy as jnp
import jax.experimental.pallas as pl
import jax.experimental.pallas.tpu as pltpu


_HQ, _DH = 32, 192
_G = 2
_NQ = 4
_NDN = 4
_R = 8
_EPS = 1e-5


def _ln(x):
    m = jnp.mean(x, axis=-1, keepdims=True)
    d = x - m
    v = jnp.mean(d * d, axis=-1, keepdims=True)
    return d / jnp.sqrt(v + _EPS)


def _rows(x):
    return jnp.broadcast_to(x, (_R, x.shape[-1])).astype(jnp.bfloat16)


@jax.jit
def pallas_sequential_preLN__sliding_block_cached__moe_arch_mod__decode_kernel(
    A_x: jax.Array,
    A_k_cache: jax.Array,
    A_v_cache: jax.Array,
    A_wq: jax.Array,
    A_wo: jax.Array,
    B_x: jax.Array,
    B_w_r: jax.Array,
    B_w_gate: jax.Array,
    B_w_up: jax.Array,
    B_w_down: jax.Array,
):
    del B_x
    B, Sq, D = A_x.shape
    Hkv, Sk, Dh = A_k_cache.shape[1:]
    F = B_w_gate.shape[1]
    assert (B, Sq) == (1, 1) and Hkv == _HQ and Dh == _DH
    W = min(4096, max(256, Sk // 4))
    S0 = Sk - W
    HD = _HQ * _DH
    GR = _G * _DH
    NG = _HQ // _G
    QC = HD // _NQ
    DC = F // _NDN
    scale = _DH ** -0.5
    f32, bf16 = jnp.float32, jnp.bfloat16

    kt = jnp.transpose(A_k_cache, (0, 1, 3, 2)).reshape(HD, Sk)
    vt = jnp.transpose(A_v_cache, (0, 1, 3, 2)).reshape(HD, Sk)

    def kernel(x_hbm, k_hbm, v_hbm, wq_hbm, wo_hbm, wr_hbm, wg_hbm, wu_hbm, wd_hbm,
               o_ref, x_v, wr_v, wq_v, k_v, v_v, wo_v, wg_v, wu_v, wd_v, q_v,
               s_small, s_q, s_k, s_v, s_o, s_f, s_d):
        x_cp = pltpu.make_async_copy(x_hbm.at[0], x_v, s_small.at[0])
        wr_cp = pltpu.make_async_copy(wr_hbm, wr_v, s_small.at[1])

        def wq_cp(c):
            return pltpu.make_async_copy(
                wq_hbm.at[:, pl.ds(c * QC, QC)], wq_v.at[c], s_q.at[c])

        def kv_cp(hbm, buf, sem, g, slot):
            r0 = g * GR if isinstance(g, int) else pl.multiple_of(g * GR, GR)
            return pltpu.make_async_copy(
                hbm.at[pl.ds(r0, GR), pl.ds(S0, W)], buf.at[slot], sem.at[slot])

        def wo_cp(g, slot):
            r0 = g * GR if isinstance(g, int) else pl.multiple_of(g * GR, GR)
            return pltpu.make_async_copy(
                wo_hbm.at[pl.ds(r0, GR), :], wo_v.at[slot], s_o.at[slot])

        wg_cp = pltpu.make_async_copy(wg_hbm, wg_v, s_f.at[0])
        wu_cp = pltpu.make_async_copy(wu_hbm, wu_v, s_f.at[1])

        def wd_cp(c):
            return pltpu.make_async_copy(
                wd_hbm.at[pl.ds(c * DC, DC), :], wd_v.at[c], s_d.at[c])

        wq_cp(0).start()
        x_cp.start()
        wq_cp(1).start()
        wr_cp.start()
        x_cp.wait()
        x = x_v[...].astype(f32)
        xn = _rows(_ln(x))
        for c in range(_NQ):
            wq_cp(c).wait()
            if c + 2 < _NQ:
                wq_cp(c + 2).start()
            elif c + 2 == _NQ:
                kv_cp(k_hbm, k_v, s_k, 0, 0).start()
            else:
                kv_cp(v_hbm, v_v, s_v, 0, 0).start()
                wo_cp(0, 0).start()
            qc = jnp.dot(xn, wq_v[c], preferred_element_type=f32)
            for j in range(QC // GR):
                q_v[c * (QC // GR) + j] = qc[:, j * GR:(j + 1) * GR]

        row = jax.lax.broadcasted_iota(jnp.int32, (_R, GR), 0)
        col = jax.lax.broadcasted_iota(jnp.int32, (_R, GR), 1)
        diag = jnp.logical_and(col >= row * _DH, col < (row + 1) * _DH)

        def group(g, acc):
            slot = g % 2
            nxt = 1 - slot
            more = g + 1 < NG
            kv_cp(k_hbm, k_v, s_k, g, slot).wait()

            @pl.when(more)
            def _():
                kv_cp(k_hbm, k_v, s_k, g + 1, nxt).start()

            @pl.when(jnp.logical_not(more))
            def _():
                wg_cp.start()

            qd = jnp.where(diag, q_v[g], 0.0).astype(bf16)
            s = jnp.dot(qd, k_v[slot], preferred_element_type=f32) * scale
            e = jnp.exp(s - jnp.max(s, axis=-1, keepdims=True))
            p = (e / jnp.sum(e, axis=-1, keepdims=True)).astype(bf16)

            kv_cp(v_hbm, v_v, s_v, g, slot).wait()
            wo_cp(g, slot).wait()

            @pl.when(more)
            def _():
                kv_cp(v_hbm, v_v, s_v, g + 1, nxt).start()
                wo_cp(g + 1, nxt).start()

            @pl.when(jnp.logical_not(more))
            def _():
                wu_cp.start()

            o = jax.lax.dot_general(p, v_v[slot], (((1,), (1,)), ((), ())),
                                    preferred_element_type=f32)
            o = jnp.sum(jnp.where(diag, o, 0.0), axis=0, keepdims=True)
            return acc + jnp.dot(_rows(o), wo_v[slot], preferred_element_type=f32)

        acc = jax.lax.fori_loop(0, NG, group, jnp.zeros((_R, D), f32))

        h = x + acc[0:1]
        hn = _ln(h)
        hb = _rows(hn)
        wr_cp.wait()
        r = jnp.sum(hb[0:1].astype(f32) * wr_v[...].astype(f32).reshape(1, D),
                    axis=-1, keepdims=True)
        gate_r = jax.nn.sigmoid(r)

        wg_cp.wait()
        for c in range(_NDN // 2):
            wd_cp(c).start()
        gt = jnp.dot(hb, wg_v[...], preferred_element_type=f32)
        gt = gt * jax.nn.sigmoid(gt)
        wu_cp.wait()
        for c in range(_NDN // 2, _NDN):
            wd_cp(c).start()
        up = jnp.dot(hb, wu_v[...], preferred_element_type=f32)
        a = (gt * up).astype(bf16)
        y = jnp.zeros((_R, D), f32)
        for c in range(_NDN):
            wd_cp(c).wait()
            y = y + jnp.dot(a[:, c * DC:(c + 1) * DC], wd_v[c],
                            preferred_element_type=f32)
        o_ref[0] = (h + (hn + y[0:1] * gate_r)).astype(o_ref.dtype)

    any_spec = pl.BlockSpec(memory_space=pl.ANY)
    dma = pltpu.SemaphoreType.DMA
    return pl.pallas_call(
        kernel,
        out_shape=jax.ShapeDtypeStruct((B, Sq, D), A_x.dtype),
        in_specs=[any_spec] * 9,
        scratch_shapes=[
            pltpu.VMEM((1, D), bf16),
            pltpu.VMEM((D,), bf16),
            pltpu.VMEM((_NQ, D, QC), bf16),
            pltpu.VMEM((2, GR, W), bf16),
            pltpu.VMEM((2, GR, W), bf16),
            pltpu.VMEM((2, GR, D), bf16),
            pltpu.VMEM((D, F), bf16),
            pltpu.VMEM((D, F), bf16),
            pltpu.VMEM((_NDN, DC, D), bf16),
            pltpu.VMEM((NG, _R, GR), f32),
            dma((2,)), dma((_NQ,)), dma((2,)), dma((2,)), dma((2,)),
            dma((2,)), dma((_NDN,)),
        ],
        compiler_params=pltpu.CompilerParams(vmem_limit_bytes=64 * 2**20),
    )(A_x, kt, vt, A_wq, A_wo, B_w_r, B_w_gate, B_w_up, B_w_down)
```
